```python
import os as _os
_os.environ.setdefault('JAX_PLATFORMS', 'cpu')
import jax
import jax.numpy as jnp

def _softmax(x, axis=-1):
    return jax.nn.softmax(x, axis=axis)

def _gelu(x):
    return jax.nn.gelu(x, approximate=True)

def _silu(x):
    return jax.nn.silu(x)

def _sigmoid(x):
    return jax.nn.sigmoid(x)

def _layernorm(x, axis=-1, eps=1e-05):
    m = jnp.mean(x, axis=axis, keepdims=True)
    v = jnp.var(x, axis=axis, keepdims=True)
    return (x - m) / jnp.sqrt(v + eps)

def _scatter_add(tgt, idx, src, axis=0):
    return tgt.at[idx].add(src)

def _segment_sum(src, seg, n):
    return jax.ops.segment_sum(src, seg, n)

class _Rng:

    def __init__(self, key):
        self._k = key

    def _next(self):
        self._k, sub = jax.random.split(self._k)
        return sub

    def normal(self, shape):
        return jax.random.normal(self._next(), shape, dtype=jnp.bfloat16)

    def randint(self, lo, hi, shape):
        return jax.random.randint(self._next(), shape, lo, hi, dtype=jnp.int32)

    def uniform(self, shape, lo=0.0, hi=1.0):
        return jax.random.uniform(self._next(), shape, jnp.bfloat16, lo, hi)

    def permutation(self, n):
        return jax.random.permutation(self._next(), n)
kernel_name = 'parallel_sum__memory_aug_recurrent_mem_tr__dense_activation_silu__prompt'

def setup_inputs():
    _rng = _Rng(jax.random.key(int.from_bytes(__import__("os").urandom(4), "little")))
    _w = lambda a: (lambda t: t.astype(jnp.bfloat16) if jnp.issubdtype(t.dtype, jnp.floating) else t)(jnp.asarray(a))

    def _A_setup():
        B, S, Dm = (1, 2048, 448)
        H, Dh = (16, 256)
        M, seg = (8, 32)
        seg = min(seg, S)
        S = S // seg * seg
        return {'x': _w((lambda *s: _rng.normal(s) * 0.05)(B, S, Dm)), 'mem0': _w((lambda *s: _rng.normal(s) * 0.2)(B, M, Dm)), 'Wq': _w((lambda *s: _rng.normal(s) * 0.8)(Dm, H, Dh) * Dm ** (-0.5)), 'Wk': _w((lambda *s: _rng.normal(s) * 0.8)(Dm, H, Dh) * Dm ** (-0.5)), 'Wv': _w((lambda *s: _rng.normal(s) * 0.2)(Dm, H, Dh) * Dm ** (-0.5)), 'Wo': _w((lambda *s: _rng.normal(s) * 0.2)(H, Dh, Dm) * (H * Dh) ** (-0.5)), 'seg_len': seg}
    _A_in = _A_setup()

    def _B_setup():
        B, S, D, F = (1, 2048, 448, 1792)
        return {'x': _w((lambda *s: _rng.normal(s) * 0.05)(B, S, D)), 'w1': _w((lambda *s: _rng.normal(s) * 0.05)(D, F) * D ** (-0.5)), 'w2': _w((lambda *s: _rng.normal(s) * 0.05)(F, D) * F ** (-0.5))}
    _B_in = _B_setup()
    return {'A_x': _A_in['x'], 'A_mem0': _A_in['mem0'], 'A_Wq': _A_in['Wq'], 'A_Wk': _A_in['Wk'], 'A_Wv': _A_in['Wv'], 'A_Wo': _A_in['Wo'], 'A_seg_len': _A_in['seg_len'], 'B_x': _B_in['x'], 'B_w1': _B_in['w1'], 'B_w2': _B_in['w2']}

def reference(A_x, A_mem0, A_Wq, A_Wk, A_Wv, A_Wo, A_seg_len, B_x, B_w1, B_w2):

    def _A_ref(x, mem0, Wq, Wk, Wv, Wo, seg_len):
        B, S, Dm = x.shape
        H, Dh = (Wq.shape[1], Wq.shape[2])
        M = mem0.shape[1]
        scale = Dh ** (-0.5)
        n_seg = S // seg_len
        L = M + seg_len
        idx = jnp.arange(L)
        mask = (idx[:, None] < M) | (idx[:, None] >= idx[None, :])
        mem = mem0
        outs = []
        for s in range(n_seg):
            xs = x[:, s * seg_len:(s + 1) * seg_len, :].copy()
            h = jnp.concatenate([mem, xs], axis=1)
            q = jnp.einsum('btd,dhe->bhte', h, Wq)
            k = jnp.einsum('btd,dhe->bhte', h, Wk)
            v = jnp.einsum('btd,dhe->bhte', h, Wv)
            scores = jnp.einsum('bhqe,bhke->bhqk', q, k) * scale
            scores = jnp.where(mask[None, None], scores, -1000000000.0)
            p = _softmax(scores, axis=-1)
            o = jnp.einsum('bhqk,bhke->bhqe', p, v)
            o = jnp.einsum('bhte,hed->btd', o, Wo)
            mem = o[:, :M, :].copy()
            outs.append(o[:, M:, :])
        return jnp.concatenate(outs, axis=1)

    def _B_ref(x, w1, w2):
        h = jnp.einsum('bsd,df->bsf', x, w1)
        h = _silu(h)
        out = jnp.einsum('bsf,fd->bsd', h, w2)
        return out
    x = A_x
    xn = _layernorm(x, axis=-1)
    return x + _A_ref(xn, A_mem0, A_Wq, A_Wk, A_Wv, A_Wo, A_seg_len) + _B_ref(xn, B_w1, B_w2)
```

```python
import functools
import jax
import jax.numpy as jnp
from jax import lax
import jax.experimental.pallas as pl
import jax.experimental.pallas.tpu as pltpu

F32 = jnp.float32
BF16 = jnp.bfloat16

def pallas_parallel_sum__memory_aug_recurrent_mem_tr__dense_activation_silu__prompt_kernel(
    A_x, A_mem0, A_Wq, A_Wk, A_Wv, A_Wo, A_seg_len, B_x, B_w1, B_w2):
    B, S, Dm = A_x.shape
    H, Dh = A_Wq.shape[1], A_Wq.shape[2]
    M = A_mem0.shape[1]
    seg = int(A_seg_len)
    n_seg = S // seg
    L = M + seg
    Fd = B_w1.shape[1]
    scale = Dh ** (-0.5)
    HD = H * Dh
    assert B == 1

    x2 = A_x.reshape(S, Dm)
    mem0 = A_mem0.reshape(M, Dm)
    wq = A_Wq.reshape(Dm, HD)
    wk = A_Wk.reshape(Dm, HD)
    wv = A_Wv.reshape(Dm, HD)
    wo = A_Wo.reshape(HD, Dm)

    CH = 256
    n_ch = S // CH

    def kernel(x_ref, mem0_ref, wq_ref, wk_ref, wv_ref, wo_ref, w1_ref, w2_ref, o_ref,
               xn_ref, acc_ref, q_ref, k_ref, v_ref, oh_ref):
        def ffn_chunk(c, carry):
            r0 = pl.multiple_of(c * CH, CH)
            rows = pl.ds(r0, CH)
            x = x_ref[rows, :].astype(F32)
            mu = jnp.mean(x, axis=-1, keepdims=True)
            xc = x - mu
            var = jnp.mean(xc * xc, axis=-1, keepdims=True)
            xn = (xc / jnp.sqrt(var + 1e-05)).astype(BF16)
            xn_ref[rows, :] = xn
            h1 = jnp.dot(xn, w1_ref[...], preferred_element_type=F32)
            h1 = h1.astype(BF16).astype(F32)
            a = (h1 * jax.nn.sigmoid(h1)).astype(BF16)
            y = jnp.dot(a, w2_ref[...], preferred_element_type=F32)
            acc_ref[rows, :] = x + y.astype(BF16).astype(F32)
            return carry
        lax.fori_loop(0, n_ch, ffn_chunk, 0)

        qi = lax.broadcasted_iota(jnp.int32, (L, L), 0)
        kj = lax.broadcasted_iota(jnp.int32, (L, L), 1)
        mask = (qi >= seg) | (kj >= seg) | (qi >= kj)

        def seg_step(s, mem):
            r0 = pl.multiple_of(s * seg, seg)
            rows = pl.ds(r0, seg)
            hx = xn_ref[rows, :]
            h = jnp.concatenate([hx, mem], axis=0)
            q_ref[...] = (jnp.dot(h, wq_ref[...], preferred_element_type=F32) * scale).astype(BF16)
            k_ref[...] = jnp.dot(h, wk_ref[...], preferred_element_type=F32).astype(BF16)
            v_ref[...] = jnp.dot(h, wv_ref[...], preferred_element_type=F32).astype(BF16)
            for hh in range(H):
                cols = slice(hh * Dh, (hh + 1) * Dh)
                qh = q_ref[:, cols]
                kh = k_ref[:, cols]
                vh = v_ref[:, cols]
                sc = lax.dot_general(qh, kh, (((1,), (1,)), ((), ())), preferred_element_type=F32)
                sc = jnp.where(mask, sc, -1000000000.0)
                mx = jnp.max(sc, axis=-1, keepdims=True)
                e = jnp.exp(sc - mx)
                den = jnp.sum(e, axis=-1, keepdims=True)
                p = (e / den).astype(BF16)
                oh_ref[:, cols] = jnp.dot(p, vh, preferred_element_type=F32).astype(BF16)
            out = jnp.dot(oh_ref[...], wo_ref[...], preferred_element_type=F32)
            acc_ref[rows, :] = acc_ref[rows, :] + out[0:seg, :].astype(BF16).astype(F32)
            return out[seg:L, :].astype(BF16)

        lax.fori_loop(0, n_seg, seg_step, mem0_ref[...])
        o_ref[...] = acc_ref[...].astype(o_ref.dtype)

    out = pl.pallas_call(
        kernel,
        out_shape=jax.ShapeDtypeStruct((S, Dm), A_x.dtype),
        scratch_shapes=[
            pltpu.VMEM((S, Dm), BF16),
            pltpu.VMEM((S, Dm), F32),
            pltpu.VMEM((L, HD), BF16),
            pltpu.VMEM((L, HD), BF16),
            pltpu.VMEM((L, HD), BF16),
            pltpu.VMEM((L, HD), BF16),
        ],
        compiler_params=pltpu.CompilerParams(vmem_limit_bytes=100 * 1024 * 1024),
    )(x2, mem0, wq, wk, wv, wo, B_w1, B_w2)
    return out.reshape(B, S, Dm)
```

```python
import functools
import jax
import jax.numpy as jnp
from jax import lax
import jax.experimental.pallas as pl
import jax.experimental.pallas.tpu as pltpu

F32 = jnp.float32
BF16 = jnp.bfloat16


def _nt(a, b):
    return lax.dot_general(a, b, (((1,), (1,)), ((), ())), preferred_element_type=F32)


def pallas_parallel_sum__memory_aug_recurrent_mem_tr__dense_activation_silu__prompt_kernel(
    A_x, A_mem0, A_Wq, A_Wk, A_Wv, A_Wo, A_seg_len, B_x, B_w1, B_w2):
    B, S, Dm = A_x.shape
    H, Dh = A_Wq.shape[1], A_Wq.shape[2]
    M = A_mem0.shape[1]
    seg = int(A_seg_len)
    n_seg = S // seg
    Fd = B_w1.shape[1]
    scale = Dh ** (-0.5)
    HD = H * Dh
    L = M + seg
    assert B == 1 and M == 8 and seg == 32 and n_seg % 2 == 0
    assert Dh % 128 == 0 and H == 16 and Dm % 64 == 0 and S % 256 == 0
    assert scale == 2.0 ** round(-0.5 * (Dh.bit_length() - 1))

    xT = A_x.reshape(S, Dm).T
    mem0 = A_mem0.reshape(M, Dm)
    wq2 = A_Wq.reshape(Dm * H, Dh)
    wk2 = A_Wk.reshape(Dm * H, Dh)
    wv2 = A_Wv.reshape(Dm * H, Dh)
    woT = jnp.transpose(A_Wo, (0, 2, 1)).reshape(H * Dm, Dh)
    w2T = B_w2.T

    CH = 256
    n_ch = S // CH
    n_pairs = n_seg // 2
    NDB = Dm // 16
    G = 4
    HG = H // G
    GW = HG * Dh

    def kernel(xT_hbm, wq_hbm, wk_hbm, wv_hbm, woT_hbm, w1_hbm, w2T_hbm, mem0_ref,
               outT_ref,
               xT_v, w1_v, w2T_v, wq_v, wk_v, wv_v, woT_v,
               wqkv_s, wo_s, xnb_s, xnf_s, accT_s, attn_s,
               qa, ka, va, qb, kb, vb, oa_s, ob_s, sems):
        srcs = (xT_hbm, w1_hbm, w2T_hbm, wq_hbm, wk_hbm, wv_hbm, woT_hbm)
        dsts = (xT_v, w1_v, w2T_v, wq_v, wk_v, wv_v, woT_v)
        copies = [pltpu.make_async_copy(s_, d_, sems.at[i]) for i, (s_, d_) in enumerate(zip(srcs, dsts))]
        for c in copies:
            c.start()

        r128 = lax.broadcasted_iota(jnp.int32, (128, 128), 0)
        c128 = lax.broadcasted_iota(jnp.int32, (128, 128), 1)
        eye = jnp.where(r128 == c128, 1.0, 0.0).astype(BF16)

        copies[0].wait()

        def ln_chunk(c, carry):
            c0 = pl.multiple_of(c * CH, CH)
            x = xT_v[:, pl.ds(c0, CH)].astype(F32)
            mu = jnp.mean(x, axis=0, keepdims=True)
            xc = x - mu
            var = jnp.mean(xc * xc, axis=0, keepdims=True)
            xnT = (xc * (1.0 / jnp.sqrt(var + 1e-05))).astype(BF16)
            accT_s[:, pl.ds(c0, CH)] = x
            for j in range(CH // 128):
                rows = _nt(eye, xnT[:, j * 128:(j + 1) * 128])
                r0 = pl.multiple_of(c0 + j * 128, 128)
                xnf_s[pl.ds(r0, 128), :] = rows
                xnb_s[pl.ds(r0, 128), :] = rows.astype(BF16)
            return carry
        lax.fori_loop(0, n_ch, ln_chunk, 0)

        copies[1].wait()
        copies[2].wait()

        def ffn_body(c):
            c0 = pl.multiple_of(c * CH, CH)
            h1 = jnp.dot(xnb_s[pl.ds(c0, CH), :], w1_v[...], preferred_element_type=F32)
            h1 = h1.astype(BF16).astype(F32)
            a = (h1 * jax.nn.sigmoid(h1)).astype(BF16)
            yT = _nt(w2T_v[...], a)
            accT_s[:, pl.ds(c0, CH)] = accT_s[:, pl.ds(c0, CH)] + yT.astype(BF16).astype(F32)

        def ffn_chunk(c, carry):
            ffn_body(c)
            return carry
        n_plain = n_ch // 2
        lax.fori_loop(0, n_plain, ffn_chunk, 0)

        for cp in copies[3:]:
            cp.wait()
        n_rel = n_ch - n_plain
        JB = NDB // n_rel + (1 if NDB % n_rel else 0)
        HB = H // n_rel

        def ffn_rel_chunk(i, carry):
            ffn_body(n_plain + i)
            for u in range(JB):
                j = jnp.minimum(i * JB + u, NDB - 1)
                r0 = pl.multiple_of(j * 256, 256)
                d0 = pl.multiple_of(j * 16, 16)
                for wi, w_v in enumerate((wq_v, wk_v, wv_v)):
                    t = jnp.swapaxes(w_v[pl.ds(r0, 256), :].reshape(16, H, Dh), 0, 1)
                    for hh in range(H):
                        wqkv_s[pl.ds(d0, 16), wi * HD + hh * Dh: wi * HD + (hh + 1) * Dh] = t[hh]
            for u in range(HB):
                hh = i * HB + u
                r0 = pl.multiple_of(hh * Dm, 64)
                k0 = pl.multiple_of(hh * Dh, Dh)
                wo_s[pl.ds(k0, Dh), :] = woT_v[pl.ds(r0, Dm), :].T
            return carry
        lax.fori_loop(0, n_rel, ffn_rel_chunk, 0)

        ri2 = lax.broadcasted_iota(jnp.int32, (2 * L, 2 * L), 0)
        ci2 = lax.broadcasted_iota(jnp.int32, (2 * L, 2 * L), 1)
        same_head = (ri2 < L) == (ci2 < L)
        ri = jnp.where(ri2 < L, ri2, ri2 - L)
        ci = jnp.where(ci2 < L, ci2, ci2 - L)

        def tok_pos(i, even):
            if even:
                return jnp.where(i < 24, i, jnp.where(i < 32, -1, i - 8))
            return jnp.where(i < seg, i, -1)

        def make_mask(even):
            tq, tk = tok_pos(ri, even), tok_pos(ci, even)
            return same_head & ((tq < 0) | (tk < 0) | (tq >= tk))
        mask_e = make_mask(True)
        mask_o = make_mask(False)

        def proj_group(g, lhs, dst_rows, dst, extra):
            n = dst_rows[1] - dst_rows[0]
            for wi in range(3):
                c0 = wi * HD + g * GW
                res = jnp.dot(lhs, wqkv_s[:, c0:c0 + GW], preferred_element_type=F32)
                for hh in range(HG):
                    cols = slice(hh * Dh, (hh + 1) * Dh)
                    hp, ho = (g * HG + hh) // 2, ((g * HG + hh) % 2) * L
                    dst[wi][hp, ho + dst_rows[0]:ho + dst_rows[1], :] = res[0:n, cols]
                    if extra is not None:
                        extra[wi][hp, ho:ho + 8, :] = res[n:n + 8, cols]

        def attn_scores(g, bufs):
            hs = slice(g * HG // 2, (g + 1) * HG // 2)
            qh = bufs[0][hs].astype(BF16)
            kh = bufs[1][hs].astype(BF16)
            return jnp.einsum('hqe,hke->hqk', qh, kh, preferred_element_type=F32)

        def attn_finish(g, sc, bufs, mask, o_dst):
            hs = slice(g * HG // 2, (g + 1) * HG // 2)
            vh = bufs[2][hs].astype(BF16)
            sc = jnp.where(mask[None], sc * scale, -1000000000.0)
            mx = jnp.max(sc, axis=-1, keepdims=True)
            e = jnp.exp(sc - mx)
            den = jnp.sum(e, axis=-1, keepdims=True)
            p = (e * (1.0 / den)).astype(BF16)
            oh = jnp.einsum('hqk,hke->hqe', p, vh, preferred_element_type=F32)
            for hh in range(HG):
                c0 = (g * HG + hh) * Dh
                o_dst[0:L, c0:c0 + Dh] = oh[hh // 2, (hh % 2) * L:(hh % 2 + 1) * L, :]

        def segment(lhs, dst_rows, bufs, extra, mask, o_s, wo_rows):
            def wo_part(g):
                return jnp.dot(o_s[wo_rows, g * GW:(g + 1) * GW].astype(BF16), wo_s[g * GW:(g + 1) * GW, :],
                               preferred_element_type=F32)
            proj_group(0, lhs, dst_rows, bufs, extra)
            for g in range(1, G):
                sc = attn_scores(g - 1, bufs)
                proj_group(g, lhs, dst_rows, bufs, extra)
                attn_finish(g - 1, sc, bufs, mask, o_s)
            sc = attn_scores(G - 1, bufs)
            out = wo_part(0)
            for g in range(1, G - 1):
                out = out + wo_part(g)
            attn_finish(G - 1, sc, bufs, mask, o_s)
            out = out + wo_part(G - 1)
            return out

        bufa, bufb = (qa, ka, va), (qb, kb, vb)

        def pair_step(p, mem):
            r0 = pl.multiple_of(p * (2 * seg), 2 * seg)

            def xrows(a, n):
                return xnf_s[pl.ds(pl.multiple_of(r0 + a, 8), n), :]

            lhs = jnp.concatenate([xrows(0, 24), mem, xrows(24, 8), xrows(32, 8)], axis=0).astype(BF16)
            out = segment(lhs, (0, L), bufa, bufb, mask_e, oa_s, slice(0, 32))
            attn_s[pl.ds(pl.multiple_of(r0, 8), 24), :] = out[0:24, :]
            mem1 = out[24:32, :].astype(BF16).astype(F32)
            ob_s[L:L + 8, :] = oa_s[32:L, :]
            lhs = jnp.concatenate([xrows(40, 24), mem1], axis=0).astype(BF16)
            out = segment(lhs, (8, L), bufb, None, mask_o, ob_s, slice(0, L + 8))
            attn_s[pl.ds(pl.multiple_of(r0 + 32, 8), 32), :] = out[0:32, :]
            attn_s[pl.ds(pl.multiple_of(r0 + 24, 8), 8), :] = out[L:L + 8, :]
            return out[32:L, :].astype(BF16).astype(F32)

        lax.fori_loop(0, n_pairs, pair_step, mem0_ref[...].astype(F32))

        def fin_chunk(c, carry):
            c0 = pl.multiple_of(c * 128, 128)
            ab = attn_s[pl.ds(c0, 128), :].astype(BF16)
            for kt in range(pl.cdiv(Dm, 128)):
                n = min(128, Dm - kt * 128)
                blkT = _nt(eye[0:n, 0:n], ab[:, kt * 128:kt * 128 + n])
                rows = slice(kt * 128, kt * 128 + n)
                outT_ref[rows, pl.ds(c0, 128)] = (accT_s[rows, pl.ds(c0, 128)] + blkT).astype(outT_ref.dtype)
            return carry
        lax.fori_loop(0, S // 128, fin_chunk, 0)

    any_spec = pl.BlockSpec(memory_space=pl.ANY)
    outT = pl.pallas_call(
        kernel,
        out_shape=jax.ShapeDtypeStruct((Dm, S), A_x.dtype),
        in_specs=[any_spec] * 7 + [pl.BlockSpec(memory_space=pltpu.VMEM)],
        out_specs=pl.BlockSpec(memory_space=pltpu.VMEM),
        scratch_shapes=[
            pltpu.VMEM((Dm, S), BF16),
            pltpu.VMEM((Dm, Fd), BF16),
            pltpu.VMEM((Dm, Fd), BF16),
            pltpu.VMEM((Dm * H, Dh), BF16),
            pltpu.VMEM((Dm * H, Dh), BF16),
            pltpu.VMEM((Dm * H, Dh), BF16),
            pltpu.VMEM((H * Dm, Dh), BF16),
            pltpu.VMEM((Dm, 3 * HD), BF16),
            pltpu.VMEM((HD, Dm), BF16),
            pltpu.VMEM((S, Dm), BF16),
            pltpu.VMEM((S, Dm), F32),
            pltpu.VMEM((Dm, S), F32),
            pltpu.VMEM((S, Dm), F32),
            *[pltpu.VMEM((H // 2, 2 * L, Dh), F32) for _ in range(6)],
            pltpu.VMEM((L, HD), F32),
            pltpu.VMEM((L + 8, HD), F32),
            pltpu.SemaphoreType.DMA((7,)),
        ],
        compiler_params=pltpu.CompilerParams(vmem_limit_bytes=110 * 1024 * 1024),
    )(xT, wq2, wk2, wv2, woT, B_w1, w2T, mem0)
    return outT.T.reshape(B, S, Dm)
```

```python
import jax
import jax.numpy as jnp
from jax import lax
import jax.experimental.pallas as pl
import jax.experimental.pallas.tpu as pltpu

F32 = jnp.float32
BF16 = jnp.bfloat16


def _nt(a, b):
    return lax.dot_general(a, b, (((1,), (1,)), ((), ())), preferred_element_type=F32)


def pallas_parallel_sum__memory_aug_recurrent_mem_tr__dense_activation_silu__prompt_kernel(
    A_x, A_mem0, A_Wq, A_Wk, A_Wv, A_Wo, A_seg_len, B_x, B_w1, B_w2):
    B, S, Dm = A_x.shape
    H, Dh = A_Wq.shape[1], A_Wq.shape[2]
    M = A_mem0.shape[1]
    seg = int(A_seg_len)
    n_seg = S // seg
    Fd = B_w1.shape[1]
    scale = Dh ** (-0.5)
    HD = H * Dh
    L = M + seg
    assert B == 1 and M == 8 and seg == 32 and n_seg % 2 == 0
    assert Dh % 128 == 0 and H == 16 and Dm % 64 == 0 and S % 256 == 0

    xT = A_x.reshape(S, Dm).T
    mem0 = A_mem0.reshape(M, Dm)
    wq2 = A_Wq.reshape(Dm * H, Dh)
    wk2 = A_Wk.reshape(Dm * H, Dh)
    wv2 = A_Wv.reshape(Dm * H, Dh)
    woT = jnp.transpose(A_Wo, (0, 2, 1)).reshape(H * Dm, Dh)
    w2T = B_w2.T

    CH = 256
    n_ch = S // CH
    n_pairs = n_seg // 2
    NDB = Dm // 16
    G = 4
    HG = H // G
    GW = HG * Dh

    def kernel(xT_hbm, wq_hbm, wk_hbm, wv_hbm, woT_hbm, w1_hbm, w2T_hbm, mem0_ref,
               outT_ref,
               xT_v, w1_v, w2T_v, wq_v, wk_v, wv_v, woT_v,
               wqkv_s, wo_s, xnb_s, xnf_s, accT_s, attn_s,
               qa, ka, va, qb, kb, vb, oa_s, ob_s, stage_s, sems, osems):
        srcs = (xT_hbm, w1_hbm, w2T_hbm, wq_hbm, wk_hbm, wv_hbm, woT_hbm)
        dsts = (xT_v, w1_v, w2T_v, wq_v, wk_v, wv_v, woT_v)
        copies = [pltpu.make_async_copy(s_, d_, sems.at[i]) for i, (s_, d_) in enumerate(zip(srcs, dsts))]
        for c in copies:
            c.start()

        r128 = lax.broadcasted_iota(jnp.int32, (128, 128), 0)
        c128 = lax.broadcasted_iota(jnp.int32, (128, 128), 1)
        eye = jnp.where(r128 == c128, 1.0, 0.0).astype(BF16)

        copies[0].wait()

        def ln_chunk(c, carry):
            c0 = pl.multiple_of(c * CH, CH)
            x = xT_v[:, pl.ds(c0, CH)].astype(F32)
            mu = jnp.mean(x, axis=0, keepdims=True)
            xc = x - mu
            var = jnp.mean(xc * xc, axis=0, keepdims=True)
            xnT = (xc * (1.0 / jnp.sqrt(var + 1e-05))).astype(BF16)
            for j in range(CH // 128):
                rows = _nt(eye, xnT[:, j * 128:(j + 1) * 128])
                r0 = pl.multiple_of(c0 + j * 128, 128)
                xnf_s[pl.ds(r0, 128), :] = rows
                xnb_s[pl.ds(r0, 128), :] = rows.astype(BF16)
            return carry
        lax.fori_loop(0, n_ch, ln_chunk, 0)

        copies[1].wait()
        copies[2].wait()

        def ffn_body(c):
            c0 = pl.multiple_of(c * CH, CH)
            h1 = jnp.dot(xnb_s[pl.ds(c0, CH), :], w1_v[...], preferred_element_type=F32)
            h1 = h1.astype(BF16).astype(F32)
            a = (h1 * jax.nn.sigmoid(h1)).astype(BF16)
            yT = _nt(w2T_v[...], a)
            accT_s[:, pl.ds(c0, CH)] = xT_v[:, pl.ds(c0, CH)].astype(F32) + yT.astype(BF16).astype(F32)

        def ffn_chunk(c, carry):
            ffn_body(c)
            return carry
        n_plain = n_ch // 2
        lax.fori_loop(0, n_plain, ffn_chunk, 0)

        for cp in copies[3:]:
            cp.wait()
        n_rel = n_ch - n_plain
        JB = NDB // n_rel + (1 if NDB % n_rel else 0)
        HB = H // n_rel

        def ffn_rel_chunk(i, carry):
            ffn_body(n_plain + i)
            for u in range(JB):
                j = jnp.minimum(i * JB + u, NDB - 1)
                r0 = pl.multiple_of(j * 256, 256)
                d0 = pl.multiple_of(j * 16, 16)
                for wi, w_v in enumerate((wq_v, wk_v, wv_v)):
                    t = jnp.swapaxes(w_v[pl.ds(r0, 256), :].reshape(16, H, Dh), 0, 1)
                    for hh in range(H):
                        wqkv_s[pl.ds(d0, 16), wi * HD + hh * Dh: wi * HD + (hh + 1) * Dh] = t[hh]
            for u in range(HB):
                hh = i * HB + u
                r0 = pl.multiple_of(hh * Dm, 64)
                k0 = pl.multiple_of(hh * Dh, Dh)
                wo_s[pl.ds(k0, Dh), :] = woT_v[pl.ds(r0, Dm), :].T
            return carry
        lax.fori_loop(0, n_rel, ffn_rel_chunk, 0)

        ri2 = lax.broadcasted_iota(jnp.int32, (2 * L, 2 * L), 0)
        ci2 = lax.broadcasted_iota(jnp.int32, (2 * L, 2 * L), 1)
        same_head = (ri2 < L) == (ci2 < L)
        ri = jnp.where(ri2 < L, ri2, ri2 - L)
        ci = jnp.where(ci2 < L, ci2, ci2 - L)

        def tok_pos(i, even):
            if even:
                return jnp.where(i < 24, i, jnp.where(i < 32, -1, i - 8))
            return jnp.where(i < seg, i, -1)

        def make_mask(even):
            tq, tk = tok_pos(ri, even), tok_pos(ci, even)
            return same_head & ((tq < 0) | (tk < 0) | (tq >= tk))
        mask_e = make_mask(True)
        mask_o = make_mask(False)

        def proj_group(g, lhs, dst_rows, dst, extra):
            n = dst_rows[1] - dst_rows[0]
            for wi in range(3):
                c0 = wi * HD + g * GW
                res = jnp.dot(lhs, wqkv_s[:, c0:c0 + GW], preferred_element_type=F32)
                for hh in range(HG):
                    cols = slice(hh * Dh, (hh + 1) * Dh)
                    hp, ho = (g * HG + hh) // 2, ((g * HG + hh) % 2) * L
                    dst[wi][hp, ho + dst_rows[0]:ho + dst_rows[1], :] = res[0:n, cols]
                    if extra is not None:
                        extra[wi][hp, ho:ho + 8, :] = res[n:n + 8, cols]

        def attn_scores(g, bufs):
            hs = slice(g * HG // 2, (g + 1) * HG // 2)
            qh = bufs[0][hs].astype(BF16)
            kh = bufs[1][hs].astype(BF16)
            return jnp.einsum('hqe,hke->hqk', qh, kh, preferred_element_type=F32)

        def attn_finish(g, sc, bufs, mask, o_dst):
            hs = slice(g * HG // 2, (g + 1) * HG // 2)
            vh = bufs[2][hs].astype(BF16)
            sc = jnp.where(mask[None], sc * scale, -1000000000.0)
            mx = jnp.max(sc, axis=-1, keepdims=True)
            e = jnp.exp(sc - mx)
            den = jnp.sum(e, axis=-1, keepdims=True)
            p = (e * (1.0 / den)).astype(BF16)
            oh = jnp.einsum('hqk,hke->hqe', p, vh, preferred_element_type=F32)
            for hh in range(HG):
                c0 = (g * HG + hh) * Dh
                o_dst[0:L, c0:c0 + Dh] = oh[hh // 2, (hh % 2) * L:(hh % 2 + 1) * L, :]

        def segment(lhs, dst_rows, bufs, extra, mask, o_s, wo_rows):
            def wo_part(g):
                return jnp.dot(o_s[wo_rows, g * GW:(g + 1) * GW].astype(BF16), wo_s[g * GW:(g + 1) * GW, :],
                               preferred_element_type=F32)
            proj_group(0, lhs, dst_rows, bufs, extra)
            for g in range(1, G):
                sc = attn_scores(g - 1, bufs)
                proj_group(g, lhs, dst_rows, bufs, extra)
                attn_finish(g - 1, sc, bufs, mask, o_s)
            sc = attn_scores(G - 1, bufs)
            out = wo_part(0)
            for g in range(1, G - 1):
                out = out + wo_part(g)
            attn_finish(G - 1, sc, bufs, mask, o_s)
            out = out + wo_part(G - 1)
            return out

        bufa, bufb = (qa, ka, va), (qb, kb, vb)

        def pair_step(p, mem):
            r0 = pl.multiple_of(p * (2 * seg), 2 * seg)

            def xrows(a, n):
                return xnf_s[pl.ds(pl.multiple_of(r0 + a, 8), n), :]

            lhs = jnp.concatenate([xrows(0, 24), mem, xrows(24, 8), xrows(32, 8)], axis=0).astype(BF16)
            out = segment(lhs, (0, L), bufa, bufb, mask_e, oa_s, slice(0, 32))
            attn_s[pl.ds(pl.multiple_of(r0, 8), 24), :] = out[0:24, :]
            mem1 = out[24:32, :].astype(BF16).astype(F32)
            ob_s[L:L + 8, :] = oa_s[32:L, :]
            lhs = jnp.concatenate([xrows(40, 24), mem1], axis=0).astype(BF16)
            out = segment(lhs, (8, L), bufb, None, mask_o, ob_s, slice(0, L + 8))
            attn_s[pl.ds(pl.multiple_of(r0 + 32, 8), 32), :] = out[0:32, :]
            attn_s[pl.ds(pl.multiple_of(r0 + 24, 8), 8), :] = out[L:L + 8, :]
            return out[32:L, :].astype(BF16).astype(F32)

        lax.fori_loop(0, n_pairs, pair_step, mem0_ref[...].astype(F32))

        def o_copy(c):
            c0 = pl.multiple_of(c * 256, 256)
            return pltpu.make_async_copy(stage_s.at[:, pl.ds(c0, 256)], outT_ref.at[:, pl.ds(c0, 256)], osems.at[c])

        def fin_chunk(c, carry):
            for half in range(2):
                c0 = pl.multiple_of(c * 256 + half * 128, 128)
                ab = attn_s[pl.ds(c0, 128), :].astype(BF16)
                for kt in range(pl.cdiv(Dm, 128)):
                    n = min(128, Dm - kt * 128)
                    blkT = _nt(eye[0:n, 0:n], ab[:, kt * 128:kt * 128 + n])
                    rows = slice(kt * 128, kt * 128 + n)
                    stage_s[rows, pl.ds(c0, 128)] = (accT_s[rows, pl.ds(c0, 128)] + blkT).astype(stage_s.dtype)
            o_copy(c).start()
            return carry
        lax.fori_loop(0, S // 256, fin_chunk, 0)
        for c in range(S // 256):
            o_copy(c).wait()

    any_spec = pl.BlockSpec(memory_space=pl.ANY)
    outT = pl.pallas_call(
        kernel,
        out_shape=jax.ShapeDtypeStruct((Dm, S), A_x.dtype),
        in_specs=[any_spec] * 7 + [pl.BlockSpec(memory_space=pltpu.VMEM)],
        out_specs=pl.BlockSpec(memory_space=pl.ANY),
        scratch_shapes=[
            pltpu.VMEM((Dm, S), BF16),
            pltpu.VMEM((Dm, Fd), BF16),
            pltpu.VMEM((Dm, Fd), BF16),
            pltpu.VMEM((Dm * H, Dh), BF16),
            pltpu.VMEM((Dm * H, Dh), BF16),
            pltpu.VMEM((Dm * H, Dh), BF16),
            pltpu.VMEM((H * Dm, Dh), BF16),
            pltpu.VMEM((Dm, 3 * HD), BF16),
            pltpu.VMEM((HD, Dm), BF16),
            pltpu.VMEM((S, Dm), BF16),
            pltpu.VMEM((S, Dm), F32),
            pltpu.VMEM((Dm, S), F32),
            pltpu.VMEM((S, Dm), F32),
            *[pltpu.VMEM((H // 2, 2 * L, Dh), F32) for _ in range(6)],
            pltpu.VMEM((L, HD), F32),
            pltpu.VMEM((L + 8, HD), F32),
            pltpu.VMEM((Dm, S), BF16),
            pltpu.SemaphoreType.DMA((7,)),
            pltpu.SemaphoreType.DMA((S // 256,)),
        ],
        compiler_params=pltpu.CompilerParams(vmem_limit_bytes=110 * 1024 * 1024),
    )(xT, wq2, wk2, wv2, woT, B_w1, w2T, mem0)
    return outT.T.reshape(B, S, Dm)
```

```python
import jax
import jax.numpy as jnp
from jax import lax
import jax.experimental.pallas as pl
import jax.experimental.pallas.tpu as pltpu

F32 = jnp.float32
BF16 = jnp.bfloat16


def _nt(a, b):
    return lax.dot_general(a, b, (((1,), (1,)), ((), ())), preferred_element_type=F32)


def pallas_parallel_sum__memory_aug_recurrent_mem_tr__dense_activation_silu__prompt_kernel(
    A_x, A_mem0, A_Wq, A_Wk, A_Wv, A_Wo, A_seg_len, B_x, B_w1, B_w2):
    B, S, Dm = A_x.shape
    H, Dh = A_Wq.shape[1], A_Wq.shape[2]
    M = A_mem0.shape[1]
    seg = int(A_seg_len)
    n_seg = S // seg
    Fd = B_w1.shape[1]
    scale = Dh ** (-0.5)
    HD = H * Dh
    L = M + seg
    assert B == 1 and M == 8 and seg == 32 and n_seg % 8 == 0
    assert Dh % 128 == 0 and H == 16 and Dm % 64 == 0 and S % 256 == 0

    xT = A_x.reshape(S, Dm).T
    mem0 = A_mem0.reshape(M, Dm)
    wq2 = A_Wq.reshape(Dm * H, Dh)
    wk2 = A_Wk.reshape(Dm * H, Dh)
    wv2 = A_Wv.reshape(Dm * H, Dh)
    woT = jnp.transpose(A_Wo, (0, 2, 1)).reshape(H * Dm, Dh)
    w2T = B_w2.T

    CH = 256
    n_ch = S // CH
    n_pairs = n_seg // 2
    NDB = Dm // 16
    G = 4
    HG = H // G
    GW = HG * Dh

    def kernel(xT_hbm, wq_hbm, wk_hbm, wv_hbm, woT_hbm, w1_hbm, w2T_hbm, mem0_ref,
               outT_ref,
               xT_v, w1_v, w2T_v, wq_v, wk_v, wv_v, woT_v,
               wqkv_s, wo_s, xnb_s, xnf_s, accT_s, attn_s,
               qa, ka, va, qb, kb, vb, oa_s, ob_s, stage_s, sems, osems):
        srcs = (xT_hbm, w1_hbm, w2T_hbm, wq_hbm, wk_hbm, wv_hbm, woT_hbm)
        dsts = (xT_v, w1_v, w2T_v, wq_v, wk_v, wv_v, woT_v)
        copies = [pltpu.make_async_copy(s_, d_, sems.at[i]) for i, (s_, d_) in enumerate(zip(srcs, dsts))]
        for c in copies:
            c.start()

        r128 = lax.broadcasted_iota(jnp.int32, (128, 128), 0)
        c128 = lax.broadcasted_iota(jnp.int32, (128, 128), 1)
        eye = jnp.where(r128 == c128, 1.0, 0.0).astype(BF16)

        copies[0].wait()

        def ln_chunk(c, carry):
            c0 = pl.multiple_of(c * CH, CH)
            x = xT_v[:, pl.ds(c0, CH)].astype(F32)
            mu = jnp.mean(x, axis=0, keepdims=True)
            xc = x - mu
            var = jnp.mean(xc * xc, axis=0, keepdims=True)
            xnT = (xc * (1.0 / jnp.sqrt(var + 1e-05))).astype(BF16)
            for j in range(CH // 128):
                rows = _nt(eye, xnT[:, j * 128:(j + 1) * 128])
                r0 = pl.multiple_of(c0 + j * 128, 128)
                xnf_s[pl.ds(r0, 128), :] = rows
                xnb_s[pl.ds(r0, 128), :] = rows.astype(BF16)
            return carry
        lax.fori_loop(0, n_ch, ln_chunk, 0)

        copies[1].wait()
        copies[2].wait()

        def ffn_body(c):
            c0 = pl.multiple_of(c * CH, CH)
            h1 = jnp.dot(xnb_s[pl.ds(c0, CH), :], w1_v[...], preferred_element_type=F32)
            h1 = h1.astype(BF16).astype(F32)
            a = (h1 * jax.nn.sigmoid(h1)).astype(BF16)
            yT = _nt(w2T_v[...], a)
            accT_s[:, pl.ds(c0, CH)] = xT_v[:, pl.ds(c0, CH)].astype(F32) + yT.astype(BF16).astype(F32)

        def ffn_chunk(c, carry):
            ffn_body(c)
            return carry
        n_plain = n_ch - 2
        lax.fori_loop(0, n_plain, ffn_chunk, 0)

        for cp in copies[3:]:
            cp.wait()
        n_rel = n_ch - n_plain
        JB = NDB // n_rel + (1 if NDB % n_rel else 0)
        HB = H // n_rel + (1 if H % n_rel else 0)

        def ffn_rel_chunk(i, carry):
            ffn_body(n_plain + i)
            for u in range(JB):
                j = jnp.minimum(i * JB + u, NDB - 1)
                r0 = pl.multiple_of(j * 256, 256)
                d0 = pl.multiple_of(j * 16, 16)
                for wi, w_v in enumerate((wq_v, wk_v, wv_v)):
                    t = jnp.swapaxes(w_v[pl.ds(r0, 256), :].reshape(16, H, Dh), 0, 1)
                    for hh in range(H):
                        wqkv_s[pl.ds(d0, 16), wi * HD + hh * Dh: wi * HD + (hh + 1) * Dh] = t[hh]
            for u in range(HB):
                hh = jnp.minimum(i * HB + u, H - 1)
                r0 = pl.multiple_of(hh * Dm, 64)
                k0 = pl.multiple_of(hh * Dh, Dh)
                wo_s[pl.ds(k0, Dh), :] = woT_v[pl.ds(r0, Dm), :].T
            return carry
        lax.fori_loop(0, n_rel, ffn_rel_chunk, 0)

        ri2 = lax.broadcasted_iota(jnp.int32, (2 * L, 2 * L), 0)
        ci2 = lax.broadcasted_iota(jnp.int32, (2 * L, 2 * L), 1)
        same_head = (ri2 < L) == (ci2 < L)
        ri = jnp.where(ri2 < L, ri2, ri2 - L)
        ci = jnp.where(ci2 < L, ci2, ci2 - L)

        def tok_pos(i, even):
            if even:
                return jnp.where(i < 24, i, jnp.where(i < 32, -1, i - 8))
            return jnp.where(i < seg, i, -1)

        def make_mask(even):
            tq, tk = tok_pos(ri, even), tok_pos(ci, even)
            return same_head & ((tq < 0) | (tk < 0) | (tq >= tk))
        mask_e = make_mask(True)
        mask_o = make_mask(False)

        def proj_group(g, lhs, dst_rows, dst, extra):
            n = dst_rows[1] - dst_rows[0]
            for wi in range(3):
                c0 = wi * HD + g * GW
                res = jnp.dot(lhs, wqkv_s[:, c0:c0 + GW], preferred_element_type=F32)
                for hh in range(HG):
                    cols = slice(hh * Dh, (hh + 1) * Dh)
                    hp, ho = (g * HG + hh) // 2, ((g * HG + hh) % 2) * L
                    dst[wi][hp, ho + dst_rows[0]:ho + dst_rows[1], :] = res[0:n, cols]
                    if extra is not None:
                        extra[wi][hp, ho:ho + 8, :] = res[n:n + 8, cols]

        def attn_scores(g, bufs):
            hs = slice(g * HG // 2, (g + 1) * HG // 2)
            qh = bufs[0][hs].astype(BF16)
            kh = bufs[1][hs].astype(BF16)
            return jnp.einsum('hqe,hke->hqk', qh, kh, preferred_element_type=F32)

        def attn_finish(g, sc, bufs, mask, o_dst):
            hs = slice(g * HG // 2, (g + 1) * HG // 2)
            vh = bufs[2][hs].astype(BF16)
            sc = jnp.where(mask[None], sc * scale, -1000000000.0)
            mx = jnp.max(sc, axis=-1, keepdims=True)
            e = jnp.exp(sc - mx)
            den = jnp.sum(e, axis=-1, keepdims=True)
            p = (e * (1.0 / den)).astype(BF16)
            oh = jnp.einsum('hqk,hke->hqe', p, vh, preferred_element_type=F32)
            for hh in range(HG):
                c0 = (g * HG + hh) * Dh
                o_dst[0:L, c0:c0 + Dh] = oh[hh // 2, (hh % 2) * L:(hh % 2 + 1) * L, :]

        def segment(lhs, dst_rows, bufs, extra, mask, o_s, wo_rows):
            def wo_part(g):
                return jnp.dot(o_s[wo_rows, g * GW:(g + 1) * GW].astype(BF16), wo_s[g * GW:(g + 1) * GW, :],
                               preferred_element_type=F32)
            proj_group(0, lhs, dst_rows, bufs, extra)
            for g in range(1, G):
                sc = attn_scores(g - 1, bufs)
                proj_group(g, lhs, dst_rows, bufs, extra)
                attn_finish(g - 1, sc, bufs, mask, o_s)
            sc = attn_scores(G - 1, bufs)
            out = wo_part(0)
            for g in range(1, G - 1):
                out = out + wo_part(g)
            attn_finish(G - 1, sc, bufs, mask, o_s)
            out = out + wo_part(G - 1)
            return out

        bufa, bufb = (qa, ka, va), (qb, kb, vb)

        def pair_step(p, mem):
            r0 = pl.multiple_of(p * (2 * seg), 2 * seg)

            def xrows(a, n):
                return xnf_s[pl.ds(pl.multiple_of(r0 + a, 8), n), :]

            lhs = jnp.concatenate([xrows(0, 24), mem, xrows(24, 8), xrows(32, 8)], axis=0).astype(BF16)
            out = segment(lhs, (0, L), bufa, bufb, mask_e, oa_s, slice(0, 32))
            attn_s[pl.ds(pl.multiple_of(r0, 8), 24), :] = out[0:24, :]
            mem1 = out[24:32, :]
            ob_s[L:L + 8, :] = oa_s[32:L, :]
            lhs = jnp.concatenate([xrows(40, 24), mem1], axis=0).astype(BF16)
            out = segment(lhs, (8, L), bufb, None, mask_o, ob_s, slice(0, L + 8))
            attn_s[pl.ds(pl.multiple_of(r0 + 32, 8), 32), :] = out[0:32, :]
            attn_s[pl.ds(pl.multiple_of(r0 + 24, 8), 8), :] = out[L:L + 8, :]
            return out[32:L, :]

        def quad_step(qq, mem):
            for u in range(4):
                mem = pair_step(4 * qq + u, mem)
            return mem
        lax.fori_loop(0, n_pairs // 4, quad_step, mem0_ref[...].astype(F32))

        def o_copy(c):
            c0 = pl.multiple_of(c * 256, 256)
            return pltpu.make_async_copy(stage_s.at[:, pl.ds(c0, 256)], outT_ref.at[:, pl.ds(c0, 256)], osems.at[c])

        def fin_chunk(c, carry):
            for half in range(2):
                c0 = pl.multiple_of(c * 256 + half * 128, 128)
                ab = attn_s[pl.ds(c0, 128), :].astype(BF16)
                for kt in range(pl.cdiv(Dm, 128)):
                    n = min(128, Dm - kt * 128)
                    blkT = _nt(eye[0:n, 0:n], ab[:, kt * 128:kt * 128 + n])
                    rows = slice(kt * 128, kt * 128 + n)
                    stage_s[rows, pl.ds(c0, 128)] = (accT_s[rows, pl.ds(c0, 128)] + blkT).astype(stage_s.dtype)
            o_copy(c).start()
            return carry
        lax.fori_loop(0, S // 256, fin_chunk, 0)
        for c in range(S // 256):
            o_copy(c).wait()

    any_spec = pl.BlockSpec(memory_space=pl.ANY)
    outT = pl.pallas_call(
        kernel,
        out_shape=jax.ShapeDtypeStruct((Dm, S), A_x.dtype),
        in_specs=[any_spec] * 7 + [pl.BlockSpec(memory_space=pltpu.VMEM)],
        out_specs=pl.BlockSpec(memory_space=pl.ANY),
        scratch_shapes=[
            pltpu.VMEM((Dm, S), BF16),
            pltpu.VMEM((Dm, Fd), BF16),
            pltpu.VMEM((Dm, Fd), BF16),
            pltpu.VMEM((Dm * H, Dh), BF16),
            pltpu.VMEM((Dm * H, Dh), BF16),
            pltpu.VMEM((Dm * H, Dh), BF16),
            pltpu.VMEM((H * Dm, Dh), BF16),
            pltpu.VMEM((Dm, 3 * HD), BF16),
            pltpu.VMEM((HD, Dm), BF16),
            pltpu.VMEM((S, Dm), BF16),
            pltpu.VMEM((S, Dm), F32),
            pltpu.VMEM((Dm, S), F32),
            pltpu.VMEM((S, Dm), F32),
            *[pltpu.VMEM((H // 2, 2 * L, Dh), F32) for _ in range(6)],
            pltpu.VMEM((L, HD), F32),
            pltpu.VMEM((L + 8, HD), F32),
            pltpu.VMEM((Dm, S), BF16),
            pltpu.SemaphoreType.DMA((7,)),
            pltpu.SemaphoreType.DMA((S // 256,)),
        ],
        compiler_params=pltpu.CompilerParams(vmem_limit_bytes=110 * 1024 * 1024),
    )(xT, wq2, wk2, wv2, woT, B_w1, w2T, mem0)
    return outT.T.reshape(B, S, Dm)
```
